```python
import os as _os
_os.environ.setdefault("JAX_PLATFORMS", "cpu")
import jax
import jax.numpy as jnp

def _softmax(x, axis=-1):
    return jax.nn.softmax(x, axis=axis)
def _gelu(x):
    return jax.nn.gelu(x, approximate=True)
def _silu(x):
    return jax.nn.silu(x)
def _sigmoid(x):
    return jax.nn.sigmoid(x)
def _layernorm(x, axis=-1, eps=1e-5):
    m = jnp.mean(x, axis=axis, keepdims=True)
    v = jnp.var(x, axis=axis, keepdims=True)
    return (x - m) / jnp.sqrt(v + eps)
def _scatter_add(tgt, idx, src, axis=0):
    return tgt.at[idx].add(src)
def _segment_sum(src, seg, n):
    return jax.ops.segment_sum(src, seg, n)
class _Rng:
    def __init__(self, key):
        self._k = key
    def _next(self):
        self._k, sub = jax.random.split(self._k)
        return sub
    def normal(self, shape):
        return jax.random.normal(self._next(), shape, dtype=jnp.bfloat16)
    def randint(self, lo, hi, shape):
        return jax.random.randint(self._next(), shape, lo, hi, dtype=jnp.int32)
    def uniform(self, shape, lo=0.0, hi=1.0):
        return jax.random.uniform(self._next(), shape, jnp.bfloat16, lo, hi)
    def permutation(self, n):
        return jax.random.permutation(self._next(), n)


kernel_name = 'standalone__sliding_block_cached__sampling'

def setup_inputs():
    _rng = _Rng(jax.random.key(int.from_bytes(__import__("os").urandom(4), "little")))
    _w = (lambda a: (lambda t: t.astype(jnp.bfloat16) if jnp.issubdtype(t.dtype, jnp.floating) else t)(jnp.asarray(a)))
    B, Sq, D = 8, 16, 576
    Hq, Hkv, Sk, Dh = 32, 16, 8192, 128
    assert Hq % Hkv == 0, (Hq, Hkv)
    return {
        "x": _w((lambda *s: _rng.normal(s) * 0.8)(B, Sq, D)),
        "k_cache": _w((lambda *s: _rng.normal(s) * 0.8)(B, Hkv, Sk, Dh)),
        "v_cache": _w((lambda *s: _rng.normal(s) * 0.05)(B, Hkv, Sk, Dh)),
        "wq": _w((lambda *s: _rng.normal(s) * 0.8)(D, Hq * Dh) * (D ** -0.5)),
        "wo": _w((lambda *s: _rng.normal(s) * 0.05)(Hq * Dh, D) * ((Hq * Dh) ** -0.5)),
    }

def reference(x, k_cache, v_cache, wq, wo):
    B, Sq, D = x.shape
    Hq, Dh = 32, 128
    Hkv, Sk = k_cache.shape[1], k_cache.shape[2]
    W = min(4096, max(256, Sk // 4))
    rep = Hq // Hkv
    q = (lambda x, *d: x.transpose(*d))((x @ wq).reshape(B, Sq, Hq, Dh), 0, 2, 1, 3)
    k = jnp.repeat(k_cache[:, :, Sk - W:, :], rep, axis=1)
    v = jnp.repeat(v_cache[:, :, Sk - W:, :], rep, axis=1)
    scores = jnp.einsum("bhqd,bhkd->bhqk", q, k) * (Dh ** -0.5)
    p = _softmax(scores, axis=-1)
    o = jnp.einsum("bhqk,bhkd->bhqd", p, v)
    return (lambda x, *d: x.transpose(*d))(o, 0, 2, 1, 3).reshape(B, Sq, Hq * Dh) @ wo
```

```python
import functools

import jax
import jax.numpy as jnp
import numpy as np
from jax import lax
import jax.experimental.pallas as pl
import jax.experimental.pallas.tpu as pltpu

HQ = 32
DH = 128
ROWS = 128
GROUP = 4
SLOTS = 2
THREAD_LAG = 56
WO_ISSUE = (80, 118)
NT = (((1,), (1,)), ((), ()))


def _interleave(items, n):
    if len(items) % n:
        return list(items)
    per = len(items) // n
    return [items[(i % n) * per + i // n] for i in range(len(items))]


def _issue_order(items):
    n = len(items)
    landing = sorted(range(n), key=lambda s: (s + THREAD_LAG * (s % 2), s))
    out = [None] * n
    for item, s in zip(items, landing):
        out[s] = (item, s % 2)
    return out


def _output_pieces(d, e):
    full = d // 128
    blocks = [(full * 128, d - full * 128, (e,))] if d % 128 else []
    for i in range(full):
        if i == full - 1:
            ks = (e // 2, e // 4, e // 4)
        elif i == full - 2:
            ks = (e // 2, e // 2)
        else:
            ks = (e,)
        blocks.append((i * 128, 128, ks))
    pieces = []
    for row0, rows, ks in blocks:
        k0 = 0
        for j, k in enumerate(ks):
            pieces.append((row0, rows, k0, k, j == 0, j == len(ks) - 1))
            k0 += k
    return pieces


@jax.jit
def pallas_standalone__sliding_block_cached__sampling_kernel(
    x: jax.Array,
    k_cache: jax.Array,
    v_cache: jax.Array,
    wq: jax.Array,
    wo: jax.Array,
):
    B, SQ, D = x.shape
    _, HKV, SK, _ = k_cache.shape
    W = min(4096, max(256, SK // 4))
    REP = HQ // HKV
    M = B * SQ
    E = HQ * DH
    assert HKV % GROUP == 0 and W % ROWS == 0 and SK % ROWS == 0
    n_groups = B * HKV // GROUP
    head_chunks = SK // ROWS
    first_chunk = (SK - W) // ROWS
    q_cols = GROUP * REP * DH
    exp2_scale = float(DH**-0.5 * np.log2(np.e))

    kv_copies = [(w, g, c) for c in range(W // ROWS) for g in range(GROUP) for w in (0, 1)]
    wq_cols = ROWS * DH // 8
    wq_copies = [(r, c) for r in range(0, D, 8) for c in range(0, E, wq_cols)]
    half = len(wq_copies) // 2
    wq_copies = [
        rc
        for pair in zip(_interleave(wq_copies[:half], 3), _interleave(wq_copies[half:], 3))
        for rc in pair
    ]
    pieces = _output_pieces(D, E)
    wo_copies = []
    for p, (row0, rows, k0, k, _, _) in enumerate(pieces):
        cols = min(k, wq_cols)
        nrow = min(rows, ROWS * DH // cols)
        block = [
            (p, r, c, nrow, cols)
            for r in range(row0, row0 + rows, nrow)
            for c in range(k0, k0 + k, cols)
        ]
        wo_copies += _interleave(block, 2)
    final_copies = _issue_order([("kv", c) for c in kv_copies] + [("wo", c) for c in wo_copies])
    n_kv = len(kv_copies)
    wo_issue = (*WO_ISSUE, len(wo_copies))

    SEM_X, SEM_WQ, SEM_KV = 0, 1, 2
    SEM_WO = SEM_KV + SLOTS
    SEM_OUT = SEM_WO + len(pieces)

    def kernel_function(
        x_hbm, k_hbm, v_hbm, wq_hbm, wo_hbm, out_hbm,
        x_v, wq_v, wo_v, kv_v, q_v, o_v, out_v, acc_v, sems,
    ):
        kv_words = kv_v.bitcast(jnp.uint32)

        def load_kv(grp, w, g):
            return pltpu.bitcast(kv_words[grp % SLOTS, w, g], kv_v.dtype)

        def start_kv(grp, w, g, c, thread):
            slot = grp % SLOTS
            chunk = grp * (GROUP * head_chunks) + (g * head_chunks + first_chunk + c)
            pltpu.make_async_copy(
                (k_hbm, v_hbm)[w].at[chunk],
                kv_v.at[slot, w, g, pl.ds(c * ROWS, ROWS), :],
                sems.at[SEM_KV + slot],
            ).start(priority=thread)

        def start_group(grp):
            for w, g, c in kv_copies:
                start_kv(grp, w, g, c, w)

        def start_final(lo, hi):
            for (kind, copy), thread in final_copies[lo:hi]:
                if kind == "kv":
                    start_kv(n_groups - 1, *copy, thread)
                else:
                    p, r, c, nrow, cols = copy
                    pltpu.make_async_copy(
                        wo_hbm.at[pl.ds(r, nrow), pl.ds(c, cols)],
                        wo_v.at[pl.ds(r, nrow), pl.ds(c, cols)],
                        sems.at[SEM_WO + p],
                    ).start(priority=thread)

        def wait_filled(buf, sem):
            pltpu.make_async_copy(buf, buf, sem).wait()

        def project_q(grp):
            c0 = pl.multiple_of(grp * q_cols, q_cols)
            q = jnp.dot(
                x_v[...], wq_v[:, pl.ds(c0, q_cols)], preferred_element_type=jnp.float32
            ).astype(q_v.dtype)
            for h in range(q_cols // DH):
                q_v[grp * (q_cols // DH) + h] = q[:, h * DH:(h + 1) * DH].reshape(B, SQ, DH)

        def scores(grp, g):
            i = grp * GROUP + g
            b, h = i // HKV, i % HKV
            q = jnp.concatenate([q_v[h * REP + r, b] for r in range(REP)], axis=0)
            s = lax.dot_general(q, load_kv(grp, 0, g), NT, preferred_element_type=jnp.float32)
            m = jnp.max(s, axis=1, keepdims=True)
            p = jnp.exp2((s - m) * exp2_scale)
            return p.astype(kv_v.dtype), jnp.sum(p, axis=1, keepdims=True)

        def values(grp, g, p, l):
            i = grp * GROUP + g
            b, h = i // HKV, i % HKV
            o = jnp.dot(p, load_kv(grp, 1, g), preferred_element_type=jnp.float32)
            o = (o / l).astype(o_v.dtype)
            for r in range(REP):
                o_v[h * REP + r, b] = o[r * SQ:(r + 1) * SQ]

        def attend(grp):
            p, l = scores(grp, 0)
            for g in range(GROUP):
                nxt = scores(grp, g + 1) if g + 1 < GROUP else (None, None)
                values(grp, g, p, l)
                p, l = nxt

        x_rows = M // 4
        for j in range(4):
            rows = pl.ds(j * x_rows, x_rows)
            pltpu.make_async_copy(x_hbm.at[rows], x_v.at[rows], sems.at[SEM_X]).start(priority=j % 2)
        for i, (r, c) in enumerate(wq_copies):
            pltpu.make_async_copy(
                wq_hbm.at[pl.ds(r, 8), pl.ds(c, wq_cols)],
                wq_v.at[pl.ds(r, 8), pl.ds(c, wq_cols)],
                sems.at[SEM_WQ],
            ).start(priority=i % 2)
        for grp in range(SLOTS):
            start_group(grp)
        wait_filled(x_v, sems.at[SEM_X])
        wait_filled(wq_v, sems.at[SEM_WQ])

        def group_step(grp, count):
            wait_filled(kv_v.at[grp % SLOTS], sems.at[SEM_KV + grp % SLOTS])
            pl.when(grp < HKV // GROUP)(functools.partial(project_q, grp))
            attend(grp)
            pl.when(grp + SLOTS < n_groups - 1)(functools.partial(start_group, grp + SLOTS))
            pl.when(grp + SLOTS == n_groups - 1)(functools.partial(start_final, 0, n_kv))
            pl.when(grp + SLOTS == n_groups)(
                functools.partial(start_final, n_kv, n_kv + wo_issue[0])
            )
            return count + 1

        count = lax.fori_loop(0, n_groups, group_step, 0)

        last_row0, last_rows = pieces[-1][:2]
        out_spans = [(0, last_row0), (last_row0 + last_rows, D), (last_row0, last_row0 + last_rows)]
        out_copies = [
            pltpu.make_async_copy(
                out_v.at[:, pl.ds(a, b - a)], out_hbm.at[:, pl.ds(a, b - a)], sems.at[SEM_OUT + j]
            )
            for j, (a, b) in enumerate(out_spans)
            if b > a
        ]

        def project_out(p):
            row0, rows, k0, k, first, last = pieces[p]
            w_piece = wo_v.at[pl.ds(row0, rows), pl.ds(k0, k)]
            wait_filled(w_piece, sems.at[SEM_WO + p])
            if p == len(pieces) - 1:
                for j, copy in enumerate(out_copies[:-1]):
                    copy.start(priority=j % 2)
            o = jnp.concatenate(
                [o_v[h].reshape(M, DH) for h in range(k0 // DH, (k0 + k) // DH)], axis=1
            )
            y = lax.dot_general(o, w_piece[...], NT, preferred_element_type=jnp.float32)
            if not first:
                y = y + acc_v[:, :rows]
            if last:
                out_v[:, pl.ds(row0, rows)] = y.astype(out_v.dtype)
            else:
                acc_v[:, :rows] = y

        for p in range(len(pieces)):
            if p + 1 < len(wo_issue):
                start_final(n_kv + wo_issue[p], n_kv + wo_issue[p + 1])
            if p + 1 < len(pieces):
                pl.when(count > 0)(functools.partial(project_out, p))
            else:
                project_out(p)
        out_copies[-1].start()
        for copy in out_copies:
            copy.wait()

    out = pl.pallas_call(
        kernel_function,
        out_shape=jax.ShapeDtypeStruct((M, D), x.dtype),
        in_specs=[pl.BlockSpec(memory_space=pltpu.HBM)] * 5,
        out_specs=pl.BlockSpec(memory_space=pltpu.HBM),
        scratch_shapes=[
            pltpu.VMEM((M, D), x.dtype),
            pltpu.VMEM((D, E), wq.dtype),
            pltpu.VMEM((D, E), wo.dtype),
            pltpu.VMEM((SLOTS, 2, GROUP, W, DH), k_cache.dtype),
            pltpu.VMEM((HQ, B, SQ, DH), x.dtype),
            pltpu.VMEM((HQ, B, SQ, DH), x.dtype),
            pltpu.VMEM((M, D), x.dtype),
            pltpu.VMEM((M, 128), jnp.float32),
            pltpu.SemaphoreType.DMA((SEM_OUT + 3,)),
        ],
        compiler_params=pltpu.CompilerParams(
            vmem_limit_bytes=48 * 1024 * 1024,
            disable_bounds_checks=True,
        ),
    )(
        x.reshape(M, D),
        k_cache.reshape(B * HKV * head_chunks, ROWS, DH),
        v_cache.reshape(B * HKV * head_chunks, ROWS, DH),
        wq,
        wo.T,
    )
    return out.reshape(B, SQ, D)
```

```python
import functools

import jax
import jax.numpy as jnp
import numpy as np
from jax import lax
import jax.experimental.pallas as pl
import jax.experimental.pallas.tpu as pltpu

HQ = 32
DH = 128
ROWS = 128
COPY = ROWS * DH
GROUP = 4
STRIDE = 8
SLOTS = 4
AHEAD = 3
BACKLOG = 28
WO_STARTED = (32, 80, 118)
NT = (((1,), (1,)), ((), ()))


def _interleave(items, n):
    per = -(-len(items) // n)
    return [items[j] for i in range(per) for j in range(i, len(items), per)]


def _start_order(items):
    landing = sorted(range(len(items)), key=lambda s: (s + 2 * BACKLOG * (s % 2), s))
    starts = [None] * len(items)
    for item, s in zip(items, landing):
        starts[s] = (item, s % 2)
    return starts


def _tile_copies(row0, rows, col0, cols):
    copies = []
    col = col0
    while col < col0 + cols:
        width = max(
            w for w in (2048, 1024, 512, 256, 128) if col % w == 0 and col + w <= col0 + cols
        )
        height = min(rows, COPY // width)
        copies += [(r, col, height, width) for r in range(row0, row0 + rows, height)]
        col += width
    return _interleave(sorted(copies), 2)


@jax.jit
def pallas_standalone__sliding_block_cached__sampling_kernel(
    x: jax.Array,
    k_cache: jax.Array,
    v_cache: jax.Array,
    wq: jax.Array,
    wo: jax.Array,
):
    B, SQ, D = x.shape
    _, HKV, SK, _ = k_cache.shape
    W = min(4096, max(256, SK // 4))
    REP = HQ // HKV
    M = B * SQ
    E = HQ * DH
    n_groups = B * HKV // GROUP
    n_chunks = W // ROWS
    head_chunks = SK // ROWS
    n_full, ragged = divmod(D, 128)
    assert HKV == 2 * STRIDE and (B * HKV) % (2 * GROUP * STRIDE) == 0
    assert W % (2 * ROWS) == 0 and SK % ROWS == 0
    assert D % 32 == 0 and n_full >= 3 and ragged > 0
    exp2_scale = float(DH**-0.5 * np.log2(np.e))

    def head(grp, g):
        j = grp // 2
        first = (j // STRIDE) * (2 * GROUP * STRIDE) + j % STRIDE
        return first + STRIDE * ((grp % 2) * GROUP + g)

    wq_copies = [(r, c) for r in range(0, D, 8) for c in range(0, E, COPY // 8)]
    n_thread0 = (len(wq_copies) - BACKLOG) // 2
    on_thread0 = _interleave(wq_copies[:n_thread0], 3)
    on_thread1 = _interleave(wq_copies[n_thread0:], 3)
    lead = len(on_thread1) - n_thread0
    wq_copies = [(copy, 1) for copy in on_thread1[:lead]]
    for pair in zip(on_thread0, on_thread1[lead:]):
        wq_copies += zip(pair, (0, 1))

    split_row, last_row = (n_full - 2) * 128, (n_full - 1) * 128
    stages = [
        (n_full * 128, ragged, 0, E, 1, 0, 0),
        (0, 128, 0, E, n_full - 2, 128, 0),
        (split_row, 128, 0, E // 2, 2, 0, E // 2),
        (last_row, 128, 0, 3 * E // 8, 2, 0, 3 * E // 8),
        (last_row, 128, 3 * E // 4, E // 4, 1, 0, 0),
    ]
    pieces = [
        (row0 + i * row_step, rows, k0 + i * k_step, k)
        for row0, rows, k0, k, count, row_step, k_step in stages
        for i in range(count)
    ]
    last_group = [("kv", (w, g, c)) for c in range(n_chunks) for g in range(GROUP) for w in (0, 1)]
    final_copies = _start_order(
        last_group
        + [("wo", (p, *copy)) for p, piece in enumerate(pieces) for copy in _tile_copies(*piece)]
    )
    final_edges = (0, *(len(last_group) + n for n in (0, *WO_STARTED)), len(final_copies))

    SEM_X, SEM_WQ, SEM_KV = 0, 1, 2
    SEM_WO = SEM_KV + SLOTS
    SEM_OUT = SEM_WO + len(pieces)

    def kernel_function(
        x_hbm, k_hbm, v_hbm, wq_hbm, wo_hbm, out_hbm,
        x_v, wq_v, wo_v, kv_v, q_v, o_v, out_v, acc_v, sems,
    ):
        def wait_filled(buf, sem):
            pltpu.make_async_copy(buf, buf, sem).wait()

        def start_kv(chunk, slot, w, g, c, thread):
            row = c * ROWS if isinstance(c, int) else pl.multiple_of(c * ROWS, ROWS)
            pltpu.make_async_copy(
                (k_hbm, v_hbm)[w].at[chunk],
                kv_v.at[slot, w, g, pl.ds(row, ROWS), :],
                sems.at[SEM_KV + slot],
            ).start(priority=thread)

        def start_groups(grp, count, c0, n):
            first = head(grp, 0) * head_chunks + (head_chunks - n_chunks) + c0
            slot = grp % SLOTS
            for c in range(n):
                for g in range(count * GROUP):
                    chunk = first + (STRIDE * g * head_chunks + c)
                    for w in (0, 1):
                        start_kv(chunk, slot + g // GROUP, w, g % GROUP, c0 + c, w)

        def start_final(part):
            grp = n_groups - 1
            for (kind, copy), thread in final_copies[final_edges[part]:final_edges[part + 1]]:
                if kind == "kv":
                    w, g, c = copy
                    chunk = (head(grp, g) + 1) * head_chunks - n_chunks + c
                    start_kv(chunk, grp % SLOTS, w, g, c, thread)
                else:
                    p, r, c, rows, cols = copy
                    pltpu.make_async_copy(
                        wo_hbm.at[pl.ds(r, rows), pl.ds(c, cols)],
                        wo_v.at[pl.ds(r, rows), pl.ds(c, cols)],
                        sems.at[SEM_WO + p],
                    ).start(priority=thread)

        def project_q(h):
            col = pl.multiple_of(h * (REP * DH), REP * DH)
            q = jnp.dot(
                x_v[...], wq_v[:, pl.ds(col, REP * DH)], preferred_element_type=jnp.float32
            ).astype(q_v.dtype)
            for r in range(REP):
                q_v[h * REP + r] = q[:, r * DH:(r + 1) * DH].reshape(B, SQ, DH)

        def scores(grp, g):
            b, h = head(grp, g) // HKV, head(grp, g) % HKV
            q = jnp.concatenate([q_v[h * REP + r, b] for r in range(REP)], axis=0)
            s = lax.dot_general(
                q, kv_v[grp % SLOTS, 0, g], NT, preferred_element_type=jnp.float32
            )
            m = jnp.max(s, axis=1, keepdims=True)
            p = jnp.exp2((s - m) * exp2_scale)
            return p.astype(kv_v.dtype), jnp.sum(p, axis=1, keepdims=True)

        def values(grp, g, p, l):
            b, h = head(grp, g) // HKV, head(grp, g) % HKV
            o = jnp.dot(p, kv_v[grp % SLOTS, 1, g], preferred_element_type=jnp.float32)
            o = (o / l).astype(o_v.dtype)
            for r in range(REP):
                o_v[h * REP + r, b] = o[r * SQ:(r + 1) * SQ]

        def attend(grp):
            wait_filled(kv_v.at[grp % SLOTS], sems.at[SEM_KV + grp % SLOTS])
            p, l = scores(grp, 0)
            for g in range(GROUP):
                following = scores(grp, g + 1) if g + 1 < GROUP else (None, None)
                values(grp, g, p, l)
                p, l = following

        for (r, c), thread in wq_copies:
            pltpu.make_async_copy(
                wq_hbm.at[pl.ds(r, 8), pl.ds(c, COPY // 8)],
                wq_v.at[pl.ds(r, 8), pl.ds(c, COPY // 8)],
                sems.at[SEM_WQ],
            ).start(priority=thread)
        for j in range(4):
            rows = pl.ds(j * (M // 4), M // 4)
            pltpu.make_async_copy(x_hbm.at[rows], x_v.at[rows], sems.at[SEM_X]).start(
                priority=j % 2
            )

        def step(i, count):
            @pl.when(i == 1)
            def _():
                wait_filled(x_v, sems.at[SEM_X])
                wait_filled(wq_v, sems.at[SEM_WQ])

            @pl.when(jnp.logical_and(i >= 1, i <= HKV))
            def _():
                project_q((i - 1) // 2 + STRIDE * ((i - 1) % 2))

            pl.when(i >= AHEAD)(lambda: attend(i - AHEAD))

            @pl.when(i < n_groups - 2)
            def _():
                half = i % 2
                start_groups(i - half, 2, half * (n_chunks // 2), n_chunks // 2)

            pl.when(i == n_groups - 2)(lambda: start_groups(n_groups - 2, 1, 0, n_chunks))
            for part in range(AHEAD):
                pl.when(i == n_groups - 1 + part)(functools.partial(start_final, part))
            return count + 1

        steps_done = lax.fori_loop(0, n_groups + AHEAD, step, 0)

        out_copies = [
            pltpu.make_async_copy(
                out_v.at[:, pl.ds(a, b - a)], out_hbm.at[:, pl.ds(a, b - a)], sems.at[SEM_OUT + j]
            )
            for j, (a, b) in enumerate(
                [(0, last_row), (last_row + 128, D), (last_row, last_row + 128)]
            )
        ]

        def project_out(stage, first_piece, i, _=None):
            row0, rows, k0, k, _, row_step, k_step = stages[stage]
            row = pl.multiple_of(row0 + i * row_step, 128) if row_step else row0
            col = pl.multiple_of(k0 + i * k_step, 128) if k_step else k0
            w_piece = wo_v.at[pl.ds(row, rows), pl.ds(col, k)]
            wait_filled(w_piece, sems.at[SEM_WO + first_piece + i])
            if stage == len(stages) - 1:
                out_copies[0].start(priority=0)
                out_copies[1].start(priority=1)
            o = jnp.concatenate(
                [o_v[col // DH + h].reshape(M, DH) for h in range(k // DH)], axis=1
            )
            y = lax.dot_general(o, w_piece[...], NT, preferred_element_type=jnp.float32)
            if k < E:
                block = (row0 - split_row) // 128
                y = y + acc_v[block]
                if stage < len(stages) - 1:
                    acc_v[block] = y
            if stage != len(stages) - 2:
                out_v[:, pl.ds(row, rows)] = y.astype(out_v.dtype)

        acc_v[...] = jnp.zeros(acc_v.shape, acc_v.dtype)
        first_piece = 0
        for stage, (*_, count, _, _) in enumerate(stages):
            if AHEAD + stage + 1 < len(final_edges):
                start_final(AHEAD + stage)
            piece = functools.partial(project_out, stage, first_piece)
            if count > 1:
                lax.fori_loop(0, count, piece, None)
            elif stage < len(stages) - 1:
                pl.when(steps_done > 0)(functools.partial(piece, 0))
            else:
                piece(0)
            first_piece += count
        out_copies[2].start()
        for copy in out_copies:
            copy.wait()

    out = pl.pallas_call(
        kernel_function,
        out_shape=jax.ShapeDtypeStruct((M, D), x.dtype),
        in_specs=[pl.BlockSpec(memory_space=pltpu.HBM)] * 5,
        out_specs=pl.BlockSpec(memory_space=pltpu.HBM),
        scratch_shapes=[
            pltpu.VMEM((M, D), x.dtype),
            pltpu.VMEM((D, E), wq.dtype),
            pltpu.VMEM((D, E), wo.dtype),
            pltpu.VMEM((SLOTS, 2, GROUP, W, DH), k_cache.dtype),
            pltpu.VMEM((HQ, B, SQ, DH), x.dtype),
            pltpu.VMEM((HQ, B, SQ, DH), x.dtype),
            pltpu.VMEM((M, D), x.dtype),
            pltpu.VMEM((2, M, 128), jnp.float32),
            pltpu.SemaphoreType.DMA((SEM_OUT + 3,)),
        ],
        compiler_params=pltpu.CompilerParams(
            vmem_limit_bytes=56 * 1024 * 1024,
            disable_bounds_checks=True,
            disable_semaphore_checks=True,
        ),
    )(
        x.reshape(M, D),
        k_cache.reshape(B * HKV * head_chunks, ROWS, DH),
        v_cache.reshape(B * HKV * head_chunks, ROWS, DH),
        wq,
        wo.T,
    )
    return out.reshape(B, SQ, D)
```

```python
import functools

import jax
import jax.numpy as jnp
import numpy as np
from jax import lax
import jax.experimental.pallas as pl
import jax.experimental.pallas.tpu as pltpu

HQ = 32
DH = 128
ROWS = 128
COPY = ROWS * DH
GROUP = 4
STRIDE = 8
SLOTS = 4
AHEAD = 3
BACKLOG = 28
WO_STARTED = (32, 80, 118)
NT = (((1,), (1,)), ((), ()))


def _interleave(items, n):
    per = -(-len(items) // n)
    return [items[j] for i in range(per) for j in range(i, len(items), per)]


def _start_order(items):
    landing = sorted(range(len(items)), key=lambda s: (s + 2 * BACKLOG * (s % 2), s))
    starts = [None] * len(items)
    for item, s in zip(items, landing):
        starts[s] = (item, s % 2)
    return starts


def _tile_copies(row0, rows, col0, cols):
    copies = []
    col = col0
    while col < col0 + cols:
        width = max(
            w for w in (2048, 1024, 512, 256, 128) if col % w == 0 and col + w <= col0 + cols
        )
        height = min(rows, COPY // width)
        copies += [(r, col, height, width) for r in range(row0, row0 + rows, height)]
        col += width
    return _interleave(sorted(copies), 2)


@jax.jit
def pallas_standalone__sliding_block_cached__sampling_kernel(
    x: jax.Array,
    k_cache: jax.Array,
    v_cache: jax.Array,
    wq: jax.Array,
    wo: jax.Array,
):
    B, SQ, D = x.shape
    _, HKV, SK, _ = k_cache.shape
    W = min(4096, max(256, SK // 4))
    REP = HQ // HKV
    M = B * SQ
    E = HQ * DH
    n_groups = B * HKV // GROUP
    n_chunks = W // ROWS
    head_chunks = SK // ROWS
    n_full, ragged = divmod(D, 128)
    assert HKV == 2 * STRIDE and (B * HKV) % (2 * GROUP * STRIDE) == 0
    assert W % (2 * ROWS) == 0 and SK % ROWS == 0
    assert D % 32 == 0 and n_full >= 3 and ragged > 0
    exp2_scale = float(DH**-0.5 * np.log2(np.e))

    def head(grp, g):
        j = grp // 2
        first = (j // STRIDE) * (2 * GROUP * STRIDE) + j % STRIDE
        return first + STRIDE * ((grp % 2) * GROUP + g)

    wq_copies = [(r, c) for r in range(0, D, 8) for c in range(0, E, COPY // 8)]
    n_thread0 = (len(wq_copies) - BACKLOG) // 2
    on_thread0 = _interleave(wq_copies[:n_thread0], 3)
    on_thread1 = _interleave(wq_copies[n_thread0:], 3)
    lead = len(on_thread1) - n_thread0
    wq_copies = [(copy, 1) for copy in on_thread1[:lead]]
    for pair in zip(on_thread0, on_thread1[lead:]):
        wq_copies += zip(pair, (0, 1))

    split_row, last_row = (n_full - 2) * 128, (n_full - 1) * 128
    stages = [
        (n_full * 128, ragged, 0, E, 1, 0, 0),
        (0, 128, 0, E, n_full - 2, 128, 0),
        (split_row, 128, 0, E // 2, 2, 0, E // 2),
        (last_row, 128, 0, 3 * E // 8, 2, 0, 3 * E // 8),
        (last_row, 128, 3 * E // 4, E // 4, 1, 0, 0),
    ]
    pieces = [
        (row0 + i * row_step, rows, k0 + i * k_step, k)
        for row0, rows, k0, k, count, row_step, k_step in stages
        for i in range(count)
    ]
    last_group = [("kv", (w, g, c)) for c in range(n_chunks) for g in range(GROUP) for w in (0, 1)]
    final_copies = _start_order(
        last_group
        + [("wo", (p, *copy)) for p, piece in enumerate(pieces) for copy in _tile_copies(*piece)]
    )
    final_edges = (0, *(len(last_group) + n for n in (0, *WO_STARTED)), len(final_copies))

    SEM_X, SEM_WQ, SEM_KV = 0, 1, 2
    SEM_WO = SEM_KV + SLOTS
    SEM_OUT = SEM_WO + len(pieces)

    def kernel_function(
        x_hbm, k_hbm, v_hbm, wq_hbm, wo_hbm, out_hbm,
        x_v, wq_v, wo_v, kv_v, q_v, o_v, out_v, acc_v, sems,
    ):
        def wait_filled(buf, sem):
            pltpu.make_async_copy(buf, buf, sem).wait()

        def start_kv(chunk, slot, w, g, c, thread):
            row = c * ROWS if isinstance(c, int) else pl.multiple_of(c * ROWS, ROWS)
            pltpu.make_async_copy(
                (k_hbm, v_hbm)[w].at[chunk],
                kv_v.at[slot, w, g, pl.ds(row, ROWS), :],
                sems.at[SEM_KV + slot],
            ).start(priority=thread)

        def start_groups(grp, count, c0, n):
            first = head(grp, 0) * head_chunks + (head_chunks - n_chunks) + c0
            slot = grp % SLOTS
            for c in range(n):
                for g in range(count * GROUP):
                    chunk = first + (STRIDE * g * head_chunks + c)
                    for w in (0, 1):
                        start_kv(chunk, slot + g // GROUP, w, g % GROUP, c0 + c, w)

        def start_final(part):
            grp = n_groups - 1
            for (kind, copy), thread in final_copies[final_edges[part]:final_edges[part + 1]]:
                if kind == "kv":
                    w, g, c = copy
                    chunk = (head(grp, g) + 1) * head_chunks - n_chunks + c
                    start_kv(chunk, grp % SLOTS, w, g, c, thread)
                else:
                    p, r, c, rows, cols = copy
                    pltpu.make_async_copy(
                        wo_hbm.at[pl.ds(r, rows), pl.ds(c, cols)],
                        wo_v.at[pl.ds(r, rows), pl.ds(c, cols)],
                        sems.at[SEM_WO + p],
                    ).start(priority=thread)

        def project_q(h):
            col = pl.multiple_of(h * (REP * DH), REP * DH)
            q = jnp.dot(
                x_v[...], wq_v[:, pl.ds(col, REP * DH)], preferred_element_type=jnp.float32
            ).astype(q_v.dtype)
            for r in range(REP):
                q_v[h * REP + r] = q[:, r * DH:(r + 1) * DH].reshape(B, SQ, DH)

        def scores(grp, g):
            b, h = head(grp, g) // HKV, head(grp, g) % HKV
            q = jnp.concatenate([q_v[h * REP + r, b] for r in range(REP)], axis=0)
            s = lax.dot_general(
                q, kv_v[grp % SLOTS, 0, g], NT, preferred_element_type=jnp.float32
            )
            m = jnp.max(s, axis=1, keepdims=True)
            p = jnp.exp2((s - m) * exp2_scale)
            return p.astype(kv_v.dtype), jnp.sum(p, axis=1, keepdims=True)

        def values(grp, g, p, l):
            b, h = head(grp, g) // HKV, head(grp, g) % HKV
            o = jnp.dot(p, kv_v[grp % SLOTS, 1, g], preferred_element_type=jnp.float32)
            o = (o / l).astype(o_v.dtype)
            for r in range(REP):
                o_v[h * REP + r, b] = o[r * SQ:(r + 1) * SQ]

        def attend(grp):
            wait_filled(kv_v.at[grp % SLOTS], sems.at[SEM_KV + grp % SLOTS])
            p, l = scores(grp, 0)
            for g in range(GROUP):
                following = scores(grp, g + 1) if g + 1 < GROUP else (None, None)
                values(grp, g, p, l)
                p, l = following

        for (r, c), thread in wq_copies:
            pltpu.make_async_copy(
                wq_hbm.at[pl.ds(r, 8), pl.ds(c, COPY // 8)],
                wq_v.at[pl.ds(r, 8), pl.ds(c, COPY // 8)],
                sems.at[SEM_WQ],
            ).start(priority=thread)
        for j in range(4):
            rows = pl.ds(j * (M // 4), M // 4)
            pltpu.make_async_copy(x_hbm.at[rows], x_v.at[rows], sems.at[SEM_X]).start(
                priority=j % 2
            )

        def step(i, _):
            @pl.when(i == 1)
            def _():
                wait_filled(x_v, sems.at[SEM_X])
                wait_filled(wq_v, sems.at[SEM_WQ])

            @pl.when(jnp.logical_and(i >= 1, i <= HKV))
            def _():
                project_q((i - 1) // 2 + STRIDE * ((i - 1) % 2))

            pl.when(i >= AHEAD)(lambda: attend(i - AHEAD))

            @pl.when(i < n_groups - 2)
            def _():
                half = i % 2
                start_groups(i - half, 2, half * (n_chunks // 2), n_chunks // 2)

            pl.when(i == n_groups - 2)(lambda: start_groups(n_groups - 2, 1, 0, n_chunks))
            for part in range(AHEAD):
                pl.when(i == n_groups - 1 + part)(functools.partial(start_final, part))

        lax.fori_loop(0, n_groups + AHEAD, step, None)
        start_final(AHEAD)

        out_copies = [
            pltpu.make_async_copy(
                out_v.at[:, pl.ds(a, b - a)], out_hbm.at[:, pl.ds(a, b - a)], sems.at[SEM_OUT + j]
            )
            for j, (a, b) in enumerate(
                [(0, last_row), (last_row + 128, D), (last_row, last_row + 128)]
            )
        ]

        def project_out(stage, first_piece, i, _=None):
            row0, rows, k0, k, _, row_step, k_step = stages[stage]
            if stage == 1:
                pl.when(i == 0)(functools.partial(start_final, AHEAD + 1))
            row = pl.multiple_of(row0 + i * row_step, 128) if row_step else row0
            col = pl.multiple_of(k0 + i * k_step, 128) if k_step else k0
            w_piece = wo_v.at[pl.ds(row, rows), pl.ds(col, k)]
            wait_filled(w_piece, sems.at[SEM_WO + first_piece + i])
            if stage == len(stages) - 1:
                out_copies[0].start(priority=0)
                out_copies[1].start(priority=1)
            o = jnp.concatenate(
                [o_v[col // DH + h].reshape(M, DH) for h in range(k // DH)], axis=1
            )
            y = lax.dot_general(o, w_piece[...], NT, preferred_element_type=jnp.float32)
            if k < E:
                block = (row0 - split_row) // 128
                y = y + acc_v[block]
                if stage < len(stages) - 1:
                    acc_v[block] = y
            if stage != len(stages) - 2:
                out_v[:, pl.ds(row, rows)] = y.astype(out_v.dtype)

        acc_v[...] = jnp.zeros(acc_v.shape, acc_v.dtype)
        first_piece = 0
        for stage, (*_, count, _, _) in enumerate(stages):
            piece = functools.partial(project_out, stage, first_piece)
            if count > 1:
                lax.fori_loop(0, count, piece, None)
            else:
                piece(0)
            first_piece += count
        out_copies[2].start()
        for copy in out_copies:
            copy.wait()

    out = pl.pallas_call(
        kernel_function,
        out_shape=jax.ShapeDtypeStruct((M, D), x.dtype),
        in_specs=[pl.BlockSpec(memory_space=pltpu.HBM)] * 5,
        out_specs=pl.BlockSpec(memory_space=pltpu.HBM),
        scratch_shapes=[
            pltpu.VMEM((M, D), x.dtype),
            pltpu.VMEM((D, E), wq.dtype),
            pltpu.VMEM((D, E), wo.dtype),
            pltpu.VMEM((SLOTS, 2, GROUP, W, DH), k_cache.dtype),
            pltpu.VMEM((HQ, B, SQ, DH), x.dtype),
            pltpu.VMEM((HQ, B, SQ, DH), x.dtype),
            pltpu.VMEM((M, D), x.dtype),
            pltpu.VMEM((2, M, 128), jnp.float32),
            pltpu.SemaphoreType.DMA((SEM_OUT + 3,)),
        ],
        compiler_params=pltpu.CompilerParams(
            vmem_limit_bytes=56 * 1024 * 1024,
            disable_bounds_checks=True,
            disable_semaphore_checks=True,
        ),
    )(
        x.reshape(M, D),
        k_cache.reshape(B * HKV * head_chunks, ROWS, DH),
        v_cache.reshape(B * HKV * head_chunks, ROWS, DH),
        wq,
        wo.T,
    )
    return out.reshape(B, SQ, D)
```
